```python
import os as _os
_os.environ.setdefault("JAX_PLATFORMS", "cpu")
import jax
import jax.numpy as jnp

def _softmax(x, axis=-1):
    return jax.nn.softmax(x, axis=axis)
def _gelu(x):
    return jax.nn.gelu(x, approximate=True)
def _silu(x):
    return jax.nn.silu(x)
def _sigmoid(x):
    return jax.nn.sigmoid(x)
def _layernorm(x, axis=-1, eps=1e-5):
    m = jnp.mean(x, axis=axis, keepdims=True)
    v = jnp.var(x, axis=axis, keepdims=True)
    return (x - m) / jnp.sqrt(v + eps)
def _scatter_add(tgt, idx, src, axis=0):
    return tgt.at[idx].add(src)
def _segment_sum(src, seg, n):
    return jax.ops.segment_sum(src, seg, n)
class _Rng:
    def __init__(self, key):
        self._k = key
    def _next(self):
        self._k, sub = jax.random.split(self._k)
        return sub
    def normal(self, shape):
        return jax.random.normal(self._next(), shape, dtype=jnp.bfloat16)
    def randint(self, lo, hi, shape):
        return jax.random.randint(self._next(), shape, lo, hi, dtype=jnp.int32)
    def uniform(self, shape, lo=0.0, hi=1.0):
        return jax.random.uniform(self._next(), shape, jnp.bfloat16, lo, hi)
    def permutation(self, n):
        return jax.random.permutation(self._next(), n)


kernel_name = 'sequential_preLN__mha_block__moe_arch_mod__prompt'

def setup_inputs():
    _rng = _Rng(jax.random.key(int.from_bytes(__import__("os").urandom(4), "little")))
    _w = (lambda a: (lambda t: t.astype(jnp.bfloat16) if jnp.issubdtype(t.dtype, jnp.floating) else t)(jnp.asarray(a)))
    def _A_setup():
        B, S, D, H = 1, 2048, 640, 32
        return {
            "x": _w((lambda *s: _rng.normal(s) * 0.05)(B, S, D)),
            "wqkv": _w((lambda *s: _rng.normal(s) * 0.05)(D, 3 * D)),
            "wo": _w((lambda *s: _rng.normal(s) * 0.05)(D, D)),
        }
    _A_in = _A_setup()

    def _B_setup():
        B, S, D, F, C = 1, 2048, 640, 1536, 1
        return {
            "x": _w((lambda *s: _rng.normal(s) * 0.05)(B, S, D)),
            "w_r": _w((lambda *s: _rng.normal(s) * 0.05)(D)),
            "w_gate": _w((lambda *s: _rng.normal(s) * 0.05)(D, F)),
            "w_up": _w((lambda *s: _rng.normal(s) * 0.05)(D, F)),
            "w_down": _w((lambda *s: _rng.normal(s) * 0.05)(F, D)),
        }
    _B_in = _B_setup()

    return {
        "A_x": _A_in["x"],
        "A_wqkv": _A_in["wqkv"],
        "A_wo": _A_in["wo"],
        "B_x": _B_in["x"],
        "B_w_r": _B_in["w_r"],
        "B_w_gate": _B_in["w_gate"],
        "B_w_up": _B_in["w_up"],
        "B_w_down": _B_in["w_down"],
    }

def reference(A_x, A_wqkv, A_wo, B_x, B_w_r, B_w_gate, B_w_up, B_w_down):
    def _A_ref(x, wqkv, wo):
        B, S, D = x.shape
        H = 32
        Dh = D // H
        qkv = (lambda x, *d: x.transpose(*d))((x @ wqkv).reshape(B, S, 3, H, Dh), 2, 0, 3, 1, 4)
        q, k, v = qkv[0], qkv[1], qkv[2]
        scores = jnp.einsum("bhqd,bhkd->bhqk", q, k) * (Dh ** -0.5)
        p = _softmax(scores, axis=-1)
        o = jnp.einsum("bhqk,bhkd->bhqd", p, v)
        return (lambda x, *d: x.transpose(*d))(o, 0, 2, 1, 3).reshape(B, S, D) @ wo

    def _B_ref(x, w_r, w_gate, w_up, w_down):
        B, S, D = x.shape
        C = 1
        r = x @ w_r
        idx = jnp.argsort(-r, axis=-1)[:, :C]
        idx_e = jnp.repeat(idx.reshape(B, C, 1), D, axis=2)
        x_sel = jnp.take_along_axis(x, idx_e, axis=1)
        g = _silu(x_sel @ w_gate)
        u = x_sel @ w_up
        y = (g * u) @ w_down
        r_sel = _sigmoid(jnp.take_along_axis(r, idx, axis=1))
        y = y * r_sel.reshape(B, C, 1)
        b_off = (jnp.arange(B) * S).reshape(B, 1)
        flat_idx = (idx + b_off).reshape(B * C)
        zero = (x * 0.0).reshape(B * S, D)
        upd = _scatter_add(zero, flat_idx, y.reshape(B * C, D), axis=0)
        return x + upd.reshape(B, S, D)

    x = A_x
    h = x + _A_ref(_layernorm(x, axis=-1), A_wqkv, A_wo)
    h2 = h + _B_ref(_layernorm(h, axis=-1), B_w_r, B_w_gate, B_w_up, B_w_down)
    return h2
```

```python
import functools
import math

import jax
import jax.numpy as jnp
from jax import lax
import jax.experimental.pallas as pl
import jax.experimental.pallas.tpu as pltpu

S = 2048
D = 640
H = 32
DH = 20
DP = 32
NG = H * DP // 128
F = 1536
TQ = 2048
NQ = S // TQ
EPS = 1e-5


def _ln(x):
    m = jnp.mean(x, axis=-1, keepdims=True)
    xc = x - m
    v = jnp.mean(xc * xc, axis=-1, keepdims=True)
    return xc * lax.rsqrt(v + EPS)


def _kernel(x_ref, wqT_ref, wk_ref, wvT_ref, woT_ref, wr_ref, wg_ref, wu_ref, wd_ref,
            o_ref, qT_s, k_s, vT_s, oT_s, best_s, brow_s, bidx_s):
    i = pl.program_id(0)

    @pl.when(i == 0)
    def _():
        xn = _ln(x_ref[...].astype(jnp.float32))
        xnT = xn.T.astype(jnp.bfloat16)
        xn = xn.astype(jnp.bfloat16)
        scale = (DH ** -0.5) * math.log2(math.e)
        for g in range(NG):
            q = jnp.dot(wqT_ref[g * 128:(g + 1) * 128, :], xnT,
                        preferred_element_type=jnp.float32)
            qT_s[g] = (q * scale).astype(jnp.bfloat16)
            k_s[g] = jnp.dot(xn, wk_ref[:, g * 128:(g + 1) * 128],
                             preferred_element_type=jnp.float32).astype(jnp.bfloat16)
            v = jnp.dot(wvT_ref[g * 128:(g + 1) * 128, :], xnT,
                        preferred_element_type=jnp.float32)
            rid = lax.broadcasted_iota(jnp.int32, (128, S), 0)
            v = jnp.where(rid % DP == DH, 1.0, v)
            vT_s[g] = v.astype(jnp.bfloat16)
        best_s[...] = jnp.full(best_s.shape, -jnp.inf, jnp.float32)
        brow_s[...] = jnp.zeros(brow_s.shape, jnp.float32)
        bidx_s[...] = jnp.zeros(bidx_s.shape, jnp.int32)

    q0 = pl.multiple_of(i * TQ, TQ)

    def head(h, carry):
        g = h // 4
        sub = h % 4
        qg = qT_s[g, :, pl.ds(q0, TQ)]
        rid = lax.broadcasted_iota(jnp.int32, (128, TQ), 0)
        qm = jnp.where(rid // DP == sub, qg, jnp.zeros_like(qg))
        sT = jnp.dot(k_s[g], qm, preferred_element_type=jnp.float32)
        m = jnp.max(sT, axis=0, keepdims=True)
        p = jnp.exp2(sT - m).astype(jnp.bfloat16)
        vh = vT_s[g, pl.ds(pl.multiple_of(sub * DP, DP), DP), :]
        oT = jnp.dot(vh, p, preferred_element_type=jnp.float32)
        oT = oT / oT[DH:DH + 1, :]
        oT_s[g, pl.ds(pl.multiple_of(sub * DP, DP), DP), :] = oT.astype(jnp.bfloat16)
        return carry

    lax.fori_loop(0, H, head, 0, unroll=2)

    oT_all = oT_s[...].reshape(H * DP, TQ)
    aT = jnp.dot(woT_ref[...], oT_all, preferred_element_type=jnp.float32)
    hblk = x_ref[pl.ds(q0, TQ), :].astype(jnp.float32) + aT.T
    hn = _ln(hblk)
    o_ref[pl.ds(q0, TQ), :] = (hblk + hn).astype(o_ref.dtype)

    hnb = hn.astype(jnp.bfloat16).astype(jnp.float32)
    r = jnp.sum(hnb * wr_ref[...], axis=-1, keepdims=True)
    rmax = jnp.max(r, axis=0, keepdims=True)
    rows = lax.broadcasted_iota(jnp.int32, (TQ, 1), 0)
    lidx = jnp.min(jnp.where(r == rmax, rows, TQ), axis=0, keepdims=True)
    better = rmax > best_s[...]
    row = jnp.sum(jnp.where(rows == lidx, hnb, 0.0), axis=0, keepdims=True)
    brow_s[...] = jnp.where(better, row, brow_s[...])
    best_s[...] = jnp.where(better, rmax, best_s[...])
    bidx_s[...] = jnp.where(better, lidx + q0, bidx_s[...])

    @pl.when(i == NQ - 1)
    def _():
        xs = jnp.broadcast_to(brow_s[...], (8, D)).astype(jnp.bfloat16)
        gt = jnp.dot(xs, wg_ref[...], preferred_element_type=jnp.float32)
        up = jnp.dot(xs, wu_ref[...], preferred_element_type=jnp.float32)
        a = (gt * jax.nn.sigmoid(gt) * up).astype(jnp.bfloat16)
        y = jnp.dot(a, wd_ref[...], preferred_element_type=jnp.float32)[0:1]
        y = y * jax.nn.sigmoid(best_s[...])
        idx = bidx_s[0, 0]
        base = pl.multiple_of((idx // 16) * 16, 16)
        blk = o_ref[pl.ds(base, 16), :].astype(jnp.float32)
        rr = lax.broadcasted_iota(jnp.int32, (16, 1), 0)
        blk = jnp.where(rr == idx - base, blk + y, blk)
        o_ref[pl.ds(base, 16), :] = blk.astype(o_ref.dtype)


@jax.jit
def pallas_sequential_preLN__mha_block__moe_arch_mod__prompt_kernel(
    A_x, A_wqkv, A_wo, B_x, B_w_r, B_w_gate, B_w_up, B_w_down,
):
    x = A_x.reshape(S, D)
    w = jnp.pad(A_wqkv.reshape(D, 3, H, DH), ((0, 0), (0, 0), (0, 0), (0, DP - DH)))
    w = w.reshape(D, 3, H * DP)
    wqT = w[:, 0].T
    wk = w[:, 1]
    wvT = w[:, 2].T
    woT = jnp.pad(A_wo.reshape(H, DH, D), ((0, 0), (0, DP - DH), (0, 0))).reshape(H * DP, D).T
    wr = B_w_r.reshape(1, D).astype(jnp.float32)

    full = lambda a: pl.BlockSpec(a.shape, lambda i: (0,) * a.ndim)
    ins = (x, wqT, wk, wvT, woT, wr, B_w_gate, B_w_up, B_w_down)
    out = pl.pallas_call(
        _kernel,
        grid=(NQ,),
        in_specs=[full(a) for a in ins],
        out_specs=pl.BlockSpec((S, D), lambda i: (0, 0)),
        out_shape=jax.ShapeDtypeStruct((S, D), jnp.bfloat16),
        scratch_shapes=[
            pltpu.VMEM((NG, 128, S), jnp.bfloat16),
            pltpu.VMEM((NG, S, 128), jnp.bfloat16),
            pltpu.VMEM((NG, 128, S), jnp.bfloat16),
            pltpu.VMEM((NG, 128, TQ), jnp.bfloat16),
            pltpu.VMEM((1, 1), jnp.float32),
            pltpu.VMEM((1, D), jnp.float32),
            pltpu.VMEM((1, 1), jnp.int32),
        ],
        compiler_params=pltpu.CompilerParams(
            dimension_semantics=("arbitrary",), vmem_limit_bytes=100 * 1024 * 1024),
    )(*ins)
    return out.reshape(1, S, D)
```
